```python
import jax
import jax.numpy as jnp

def _softmax(x, axis=-1):
    return jax.nn.softmax(x, axis=axis)
def _gelu(x):
    return jax.nn.gelu(x, approximate=True)
def _silu(x):
    return jax.nn.silu(x)
def _sigmoid(x):
    return jax.nn.sigmoid(x)
def _layernorm(x, axis=-1, eps=1e-5):
    m = jnp.mean(x, axis=axis, keepdims=True)
    v = jnp.var(x, axis=axis, keepdims=True)
    return (x - m) / jnp.sqrt(v + eps)
def _scatter_add(tgt, idx, src, axis=0):
    return tgt.at[idx].add(src)
def _segment_sum(src, seg, n):
    return jax.ops.segment_sum(src, seg, n)
class _Rng:
    def __init__(self, key):
        self._k = key
    def _next(self):
        self._k, sub = jax.random.split(self._k)
        return sub
    def normal(self, shape):
        return jax.random.normal(self._next(), shape, dtype=jnp.bfloat16)
    def randint(self, lo, hi, shape):
        return jax.random.randint(self._next(), shape, lo, hi, dtype=jnp.int32)
    def uniform(self, shape, lo=0.0, hi=1.0):
        return jax.random.uniform(self._next(), shape, jnp.bfloat16, lo, hi)
    def permutation(self, n):
        return jax.random.permutation(self._next(), n)


kernel_name = 'sequential_preLN__spectral_gfnet__swiglu_ffn__prompt'

def _fwd_setup_inputs():
    _rng = _Rng(jax.random.key(int.from_bytes(__import__("os").urandom(4), "little")))
    _w = (lambda a: (lambda t: t.astype(jnp.bfloat16) if jnp.issubdtype(t.dtype, jnp.floating) else t)(jnp.asarray(a)))
    def _A_setup():
        B, S, D = 1, 2048, 576
        Df = D // 2 + 1
        return {
            "x": _w((lambda *s: _rng.normal(s) * 0.05)(B, S, D)),
            "w_r": _w((lambda *s: _rng.normal(s) * 0.05)(S, Df) * 0.02),
            "w_i": _w((lambda *s: _rng.normal(s) * 0.05)(S, Df) * 0.02),
        }
    _A_in = _A_setup()

    def _B_setup():
        B, S, D, F = 1, 2048, 576, 4608
        return {
            "x": _w((lambda *s: _rng.normal(s) * 0.05)(B, S, D)),
            "w_gate": _w((lambda *s: _rng.normal(s) * 0.05)(D, F)),
            "w_up": _w((lambda *s: _rng.normal(s) * 0.05)(D, F)),
            "w_down": _w((lambda *s: _rng.normal(s) * 0.05)(F, D)),
        }
    _B_in = _B_setup()

    return {
        "A_x": _A_in["x"],
        "A_w_r": _A_in["w_r"],
        "A_w_i": _A_in["w_i"],
        "B_x": _B_in["x"],
        "B_w_gate": _B_in["w_gate"],
        "B_w_up": _B_in["w_up"],
        "B_w_down": _B_in["w_down"],
    }

def _fwd_reference(A_x, A_w_r, A_w_i, B_x, B_w_gate, B_w_up, B_w_down):
    def _A_ref(x, w_r, w_i):
        B, S, D = x.shape
        X = (lambda x, axes=(-2,-1): jnp.fft.rfft2(x.astype(jnp.float32), axes=axes))(x, axes=(-2, -1))
        W = w_r + 1j * w_i
        X = X * W
        y = (lambda x, s, axes=(-2,-1): jnp.fft.irfft2(x, s=s, axes=axes).astype(jnp.bfloat16))(X, (S, D), axes=(-2, -1))
        return y

    def _B_ref(x, w_gate, w_up, w_down):
        g = _silu(x @ w_gate)
        u = x @ w_up
        return (g * u) @ w_down

    x = A_x
    h = x + _A_ref(_layernorm(x, axis=-1), A_w_r, A_w_i)
    h2 = h + _B_ref(_layernorm(h, axis=-1), B_w_gate, B_w_up, B_w_down)
    return h2


def setup_inputs():
    _inp = _fwd_setup_inputs()
    _gk = jax.random.fold_in(jax.random.key(int.from_bytes(__import__("os").urandom(4), "little")), 2**31 - 1)
    _shapes = [[1, 2048, 576]]
    _dtypes = ['bfloat16']
    _gks = jax.random.split(_gk, len(_shapes))
    _gs = [jax.random.normal(k, s, dtype=jnp.dtype(d)) * 0.05 for k, s, d in zip(_gks, _shapes, _dtypes)]
    _inp["grad_out"] = _gs[0]
    return _inp

def reference(A_x, A_w_r, A_w_i, B_w_gate, B_w_up, B_w_down, B_x, grad_out):
    _const = dict(B_x=B_x)
    def _f(*_d):
        return _fwd_reference(**{'A_x': _d[0], 'A_w_r': _d[1], 'A_w_i': _d[2], 'B_w_gate': _d[3], 'B_w_up': _d[4], 'B_w_down': _d[5], **_const})
    _out, _vjp = jax.vjp(_f, A_x, A_w_r, A_w_i, B_w_gate, B_w_up, B_w_down)
    _grads = _vjp(grad_out)
    _out0 = jnp.asarray(_out)
    return (_out0, *[jnp.asarray(_g) for _g in _grads])
```

```python
import functools
import math

import numpy as np
import jax
import jax.numpy as jnp
from jax import lax
import jax.experimental.pallas as pl
import jax.experimental.pallas.tpu as pltpu

S = 2048
D = 576
F = 4608
DF = D // 2 + 1
KP = 304
KL = 384
NB = 16
BL = 128
NL = KL // 128
EPS = 1e-5

FT = 512
TM = 256
NF = F // FT
CC = 512

f32 = jnp.float32
bf16 = jnp.bfloat16


def _make_consts():
    k = np.arange(DF)[:, None]
    d = np.arange(D)[None, :]
    ang = 2.0 * np.pi * ((d * k) % D) / D
    cs = np.zeros((2 * KP, D), np.float64)
    cs[:DF] = np.cos(ang)
    cs[KP:KP + DF] = -np.sin(ang)
    g = np.zeros((NB, 2 * BL, 2 * BL), np.float64)
    b = np.arange(BL)[:, None]
    e = np.arange(BL)[None, :]
    for c in range(NB):
        th = 2.0 * np.pi * ((b * (c + NB * e)) % S) / S
        cm, sm = np.cos(th), np.sin(th)
        g[c, :BL, :BL] = cm
        g[c, :BL, BL:] = -sm
        g[c, BL:, :BL] = sm
        g[c, BL:, BL:] = cm
    ck = np.zeros((KP, BL), np.float64)
    ck[:DF] = 2.0
    ck[0] = 1.0
    ck[DF - 1] = 1.0
    ck = ck / (S * D)
    return (cs.astype(np.float32), np.ascontiguousarray(cs.T).astype(np.float32),
            g.astype(np.float32), ck.astype(np.float32))


_CS, _CST, _G, _CK = _make_consts()


def _cmul_const(z, k, n, sign):
    re, im = z
    k = k % n
    if k == 0:
        return re, im
    if 4 * k == n:
        return (-im, re) if sign > 0 else (im, -re)
    wr = math.cos(2.0 * math.pi * k / n)
    wi = sign * math.sin(2.0 * math.pi * k / n)
    if 8 * k == n:
        c = wr
        if sign > 0:
            return (re - im) * c, (re + im) * c
        return (re + im) * c, (im - re) * c
    if 8 * k == 3 * n:
        c = -wr
        if sign > 0:
            return (-re - im) * c, (re - im) * c
        return (im - re) * c, (-re - im) * c
    return re * wr - im * wi, re * wi + im * wr


def _fft_list(xs, sign):
    n = len(xs)
    if n == 1:
        return xs
    ev = _fft_list(xs[0::2], sign)
    od = _fft_list(xs[1::2], sign)
    out = [None] * n
    for k in range(n // 2):
        tr, ti = _cmul_const(od[k], k, n, sign)
        er, ei = ev[k]
        out[k] = (er + tr, ei + ti)
        out[k + n // 2] = (er - tr, ei - ti)
    return out


def _dot(a, b):
    return jnp.dot(a, b, preferred_element_type=f32)


def _dot_nt(a, b):
    return lax.dot_general(a, b, (((1,), (1,)), ((), ())), preferred_element_type=f32)


def _ln_stats(x):
    m = jnp.mean(x, axis=0, keepdims=True)
    xc = x - m
    v = jnp.mean(xc * xc, axis=0, keepdims=True)
    return xc, lax.rsqrt(v + EPS)


def _ln_bwd(dn, n, r):
    m1 = jnp.mean(dn, axis=0, keepdims=True)
    m2 = jnp.mean(dn * n, axis=0, keepdims=True)
    return r * (dn - m1 - n * m2)


def _radix16(src_ref, dst_ref, sign, src_blocked, dst_blocked):
    def body(j, carry):
        r0 = pl.multiple_of(j * 8, 8)
        xs = []
        for a in range(NB):
            if src_blocked:
                re = src_ref[a, pl.ds(r0, 8), pl.ds(0, BL)]
                im = src_ref[a, pl.ds(r0, 8), pl.ds(BL, BL)]
            else:
                re = src_ref[pl.ds(r0, 8), pl.ds(a * BL, BL)]
                im = src_ref[pl.ds(KP + r0, 8), pl.ds(a * BL, BL)]
            xs.append((re, im))
        ys = _fft_list(xs, sign)
        for c in range(NB):
            re, im = ys[c]
            if dst_blocked:
                dst_ref[c, pl.ds(r0, 8), pl.ds(0, BL)] = re
                dst_ref[c, pl.ds(r0, 8), pl.ds(BL, BL)] = im
            else:
                dst_ref[pl.ds(r0, 8), pl.ds(c * BL, BL)] = re
                dst_ref[pl.ds(KP + r0, 8), pl.ds(c * BL, BL)] = im
        return carry
    lax.fori_loop(0, KP // 8, body, 0)


def _kernel(x_ref, wr_ref, wi_ref, wg_ref, wu_ref, wdt_ref, go_ref,
            cs_ref, cst_ref, g_ref, ck_ref,
            h2_ref, dx_ref, dwr_ref, dwi_ref, dwg_ref, dwu_ref, dwdt_ref,
            flat_s, blk_s, xsp_s, wp_s, tmp_s, pad_s, h_s, n2_s, n2t_s, gon_s,
            ft_s, dn2t_s, dwg_s, dwu_s, dwdt_s):
    step = pl.program_id(0)

    @pl.when(step == 0)
    def _phase_a():
        for p, w_ref in enumerate((wr_ref, wi_ref)):
            for l in range(NL):
                lo = l * 128
                n = min(128, DF - lo)
                if n < 128:
                    pad_s[...] = jnp.zeros(pad_s.shape, f32)
                    pad_s[pl.ds(0, n), :] = w_ref[pl.ds(lo, n), :].astype(f32)
                    tmp_s[l] = pad_s[...].T
                else:
                    tmp_s[l] = w_ref[pl.ds(lo, 128), :].astype(f32).T
            for c in range(NB):
                for l in range(NL):
                    wp_s[p, c, pl.ds(l * 128, 128), :] = tmp_s[l, pl.ds(c, BL, stride=NB), :].T

        def ln1(j, carry):
            c0 = pl.multiple_of(j * CC, CC)
            x = x_ref[0, :, pl.ds(c0, CC)].astype(f32)
            xc, r = _ln_stats(x)
            n1 = (xc * r).astype(bf16)
            flat_s[:, pl.ds(c0, CC)] = _dot(cs_ref[...], n1)
            return carry
        lax.fori_loop(0, S // CC, ln1, 0)

        _radix16(flat_s, blk_s, -1, False, True)

        def spec(c, carry):
            ck = ck_ref[...]
            xx = _dot(blk_s[c].astype(bf16), g_ref[c])
            xsp_s[c, pl.ds(0, KP), :] = xx
            xr, xi = xx[:, :BL], xx[:, BL:]
            wr = wp_s[0, c, pl.ds(0, KP), :] * ck
            wi = wp_s[1, c, pl.ds(0, KP), :] * ck
            yr = xr * wr - xi * wi
            yi = xr * wi + xi * wr
            y = jnp.concatenate([yr, yi], axis=1).astype(bf16)
            blk_s[c] = _dot_nt(y, g_ref[c])
            return carry
        lax.fori_loop(0, NB, spec, 0)

        _radix16(blk_s, flat_s, 1, True, False)

        def ln2(j, carry):
            c0 = pl.multiple_of(j * CC, CC)
            v = flat_s[:, pl.ds(c0, CC)].astype(bf16)
            y = _dot(cst_ref[...], v)
            h = x_ref[0, :, pl.ds(c0, CC)].astype(f32) + y
            h_s[:, pl.ds(c0, CC)] = h
            hc, r = _ln_stats(h)
            n2 = hc * r
            n2t_s[:, pl.ds(c0, CC)] = n2.astype(bf16)
            n2_s[pl.ds(c0, CC), :] = n2.T.astype(bf16)
            gon_s[pl.ds(c0, CC), :] = go_ref[0, :, pl.ds(c0, CC)].astype(f32).T.astype(bf16)
            return carry
        lax.fori_loop(0, S // CC, ln2, 0)

        ft_s[...] = jnp.zeros(ft_s.shape, f32)
        dn2t_s[...] = jnp.zeros(dn2t_s.shape, f32)

    dwg_s[...] = jnp.zeros(dwg_s.shape, f32)
    dwu_s[...] = jnp.zeros(dwu_s.shape, f32)
    dwdt_s[...] = jnp.zeros(dwdt_s.shape, f32)

    def chunk(j, carry):
        r0 = pl.multiple_of(j * TM, TM)
        n2c = n2_s[pl.ds(r0, TM), :]
        goc = gon_s[pl.ds(r0, TM), :]
        wg = wg_ref[...]
        wu = wu_ref[...]
        wdt = wdt_ref[...]
        a = _dot(n2c, wg)
        u = _dot(n2c, wu)
        dgu = _dot(goc, wdt)
        sig = jax.nn.sigmoid(a)
        g = a * sig
        gu = (g * u).astype(bf16)
        du = (dgu * g).astype(bf16)
        da = (dgu * u * (sig * (1.0 + a * (1.0 - sig)))).astype(bf16)
        ft_s[:, pl.ds(r0, TM)] += _dot_nt(wdt, gu)
        dn2t_s[:, pl.ds(r0, TM)] += _dot_nt(wg, da) + _dot_nt(wu, du)
        n2tc = n2t_s[:, pl.ds(r0, TM)]
        dwg_s[...] += _dot(n2tc, da)
        dwu_s[...] += _dot(n2tc, du)
        dwdt_s[...] += _dot(go_ref[0, :, pl.ds(r0, TM)], gu)
        return carry
    lax.fori_loop(0, S // TM, chunk, 0)

    dwg_ref[...] = dwg_s[...].astype(bf16)
    dwu_ref[...] = dwu_s[...].astype(bf16)
    dwdt_ref[...] = dwdt_s[...].astype(bf16)

    @pl.when(step == NF - 1)
    def _phase_c():
        def ln2b(j, carry):
            c0 = pl.multiple_of(j * CC, CC)
            h = h_s[:, pl.ds(c0, CC)]
            h2_ref[0, :, pl.ds(c0, CC)] = (h + ft_s[:, pl.ds(c0, CC)]).astype(bf16)
            hc, r = _ln_stats(h)
            dn2 = dn2t_s[:, pl.ds(c0, CC)]
            dh = go_ref[0, :, pl.ds(c0, CC)].astype(f32) + _ln_bwd(dn2, hc * r, r)
            h_s[:, pl.ds(c0, CC)] = dh
            flat_s[:, pl.ds(c0, CC)] = _dot(cs_ref[...], dh.astype(bf16))
            return carry
        lax.fori_loop(0, S // CC, ln2b, 0)

        _radix16(flat_s, blk_s, -1, False, True)

        def specb(c, carry):
            ck = ck_ref[...]
            gy = _dot(blk_s[c].astype(bf16), g_ref[c])
            gyr = gy[:, :BL] * ck
            gyi = gy[:, BL:] * ck
            xx = xsp_s[c, pl.ds(0, KP), :]
            xr, xi = xx[:, :BL], xx[:, BL:]
            wr = wp_s[0, c, pl.ds(0, KP), :]
            wi = wp_s[1, c, pl.ds(0, KP), :]
            dwr = gyr * xr + gyi * xi
            dwi = gyi * xr - gyr * xi
            xsp_s[c, pl.ds(0, KP), :] = jnp.concatenate([dwr, dwi], axis=1)
            xsp_s[c, pl.ds(KP, KL - KP), :] = jnp.zeros((KL - KP, 2 * BL), f32)
            gxr = gyr * wr + gyi * wi
            gxi = gyi * wr - gyr * wi
            gx = jnp.concatenate([gxr, gxi], axis=1).astype(bf16)
            blk_s[c] = _dot_nt(gx, g_ref[c])
            return carry
        lax.fori_loop(0, NB, specb, 0)

        for p, o_ref in enumerate((dwr_ref, dwi_ref)):
            for c in range(NB):
                for l in range(NL):
                    tmp_s[l, pl.ds(c, BL, stride=NB), :] = (
                        xsp_s[c, pl.ds(l * 128, 128), pl.ds(p * BL, BL)].T)
            for l in range(NL):
                lo = l * 128
                n = min(128, DF - lo)
                o_ref[pl.ds(lo, n), :] = tmp_s[l].T[:n].astype(bf16)

        _radix16(blk_s, flat_s, 1, True, False)

        def ln1b(j, carry):
            c0 = pl.multiple_of(j * CC, CC)
            gz = flat_s[:, pl.ds(c0, CC)].astype(bf16)
            dn1 = _dot(cst_ref[...], gz)
            x = x_ref[0, :, pl.ds(c0, CC)].astype(f32)
            xc, r = _ln_stats(x)
            dx = h_s[:, pl.ds(c0, CC)] + _ln_bwd(dn1, xc * r, r)
            dx_ref[0, :, pl.ds(c0, CC)] = dx.astype(bf16)
            return carry
        lax.fori_loop(0, S // CC, ln1b, 0)


@jax.jit
def pallas_sequential_preLN__spectral_gfnet__swiglu_ffn__prompt_kernel(
    A_x: jax.Array,
    A_w_r: jax.Array,
    A_w_i: jax.Array,
    B_x: jax.Array,
    B_w_gate: jax.Array,
    B_w_up: jax.Array,
    B_w_down: jax.Array,
    grad_out: jax.Array,
):
    del B_x
    cs = jnp.asarray(_CS, dtype=bf16)
    cst = jnp.asarray(_CST, dtype=bf16)
    g = jnp.asarray(_G, dtype=bf16)
    ck = jnp.asarray(_CK, dtype=f32)

    xt = jnp.swapaxes(A_x, 1, 2)
    got = jnp.swapaxes(grad_out, 1, 2)
    wrt = A_w_r.T
    wit = A_w_i.T
    wdt = B_w_down.T

    def whole(shape):
        nd = len(shape)
        return pl.BlockSpec(shape, lambda i: (0,) * nd, pipeline_mode=pl.Buffered(1))

    in_specs = [
        whole((1, D, S)),
        whole((DF, S)),
        whole((DF, S)),
        pl.BlockSpec((D, FT), lambda i: (0, i)),
        pl.BlockSpec((D, FT), lambda i: (0, i)),
        pl.BlockSpec((D, FT), lambda i: (0, i)),
        whole((1, D, S)),
        whole((2 * KP, D)),
        whole((D, 2 * KP)),
        whole((NB, 2 * BL, 2 * BL)),
        whole((KP, BL)),
    ]
    out_specs = [
        pl.BlockSpec((1, D, S), lambda i: (0, 0, 0)),
        pl.BlockSpec((1, D, S), lambda i: (0, 0, 0)),
        pl.BlockSpec((DF, S), lambda i: (0, 0)),
        pl.BlockSpec((DF, S), lambda i: (0, 0)),
        pl.BlockSpec((D, FT), lambda i: (0, i)),
        pl.BlockSpec((D, FT), lambda i: (0, i)),
        pl.BlockSpec((D, FT), lambda i: (0, i)),
    ]
    out_shape = [
        jax.ShapeDtypeStruct((1, D, S), bf16),
        jax.ShapeDtypeStruct((1, D, S), bf16),
        jax.ShapeDtypeStruct((DF, S), bf16),
        jax.ShapeDtypeStruct((DF, S), bf16),
        jax.ShapeDtypeStruct((D, F), bf16),
        jax.ShapeDtypeStruct((D, F), bf16),
        jax.ShapeDtypeStruct((D, F), bf16),
    ]
    scratch = [
        pltpu.VMEM((2 * KP, S), f32),
        pltpu.VMEM((NB, KP, 2 * BL), f32),
        pltpu.VMEM((NB, KL, 2 * BL), f32),
        pltpu.VMEM((2, NB, KL, BL), f32),
        pltpu.VMEM((NL, S, 128), f32),
        pltpu.VMEM((128, S), f32),
        pltpu.VMEM((D, S), f32),
        pltpu.VMEM((S, D), bf16),
        pltpu.VMEM((D, S), bf16),
        pltpu.VMEM((S, D), bf16),
        pltpu.VMEM((D, S), f32),
        pltpu.VMEM((D, S), f32),
        pltpu.VMEM((D, FT), f32),
        pltpu.VMEM((D, FT), f32),
        pltpu.VMEM((D, FT), f32),
    ]
    h2t, dxt, dwrt, dwit, dwg, dwu, dwdt = pl.pallas_call(
        _kernel,
        grid=(NF,),
        in_specs=in_specs,
        out_specs=out_specs,
        out_shape=out_shape,
        scratch_shapes=scratch,
        compiler_params=pltpu.CompilerParams(
            dimension_semantics=("arbitrary",),
            vmem_limit_bytes=110 * 1024 * 1024,
        ),
    )(xt, wrt, wit, B_w_gate, B_w_up, wdt, got, cs, cst, g, ck)
    return (jnp.swapaxes(h2t, 1, 2), jnp.swapaxes(dxt, 1, 2), dwrt.T, dwit.T,
            dwg, dwu, dwdt.T)
```

```python
import math

import numpy as np
import jax
import jax.numpy as jnp
from jax import lax
import jax.experimental.pallas as pl
import jax.experimental.pallas.tpu as pltpu

S = 2048
D = 576
F = 4608
DH = D // 2
DF = D // 2 + 1
KE = 160
KO = 144
KP = KE + KO
KL = 384
NB = 16
BL = 128
NL = KL // 128
EPS = 1e-5

FT = 512
TM = 512
NF = F // FT
CC = 1024
NCC = S // CC

f32 = jnp.float32
bf16 = jnp.bfloat16


def _make_consts():
    d = np.arange(DH)[None, :]
    ke = np.arange(0, DF, 2)[:, None]
    ko = np.arange(1, DF, 2)[:, None]
    ae = 2.0 * np.pi * ((d * ke) % D) / D
    ao = 2.0 * np.pi * ((d * ko) % D) / D
    cse = np.zeros((2 * KE, DH), np.float64)
    cse[:ke.shape[0]] = np.cos(ae)
    cse[KE:KE + ke.shape[0]] = -np.sin(ae)
    cso = np.concatenate([np.cos(ao), -np.sin(ao)], axis=0)
    g = np.zeros((NB, 2 * BL, 2 * BL), np.float64)
    b = np.arange(BL)[:, None]
    e = np.arange(BL)[None, :]
    for c in range(NB):
        th = 2.0 * np.pi * ((b * (c + NB * e)) % S) / S
        cm, sm = np.cos(th), np.sin(th)
        g[c, :BL, :BL] = cm
        g[c, :BL, BL:] = -sm
        g[c, BL:, :BL] = sm
        g[c, BL:, BL:] = cm
    ck = np.zeros((KP, BL), np.float64)
    ck[:ke.shape[0]] = 2.0
    ck[KE:] = 2.0
    ck[0] = 1.0
    ck[ke.shape[0] - 1] = 1.0
    ck = ck / (S * D)
    c32 = lambda a: np.ascontiguousarray(a).astype(np.float32)
    return c32(cse), c32(cso), c32(cse.T), c32(cso.T), c32(g), c32(ck)


_CSE, _CSO, _CSET, _CSOT, _G, _CK = _make_consts()


def _cmul_const(z, k, n, sign):
    re, im = z
    k = k % n
    if k == 0:
        return re, im
    if 4 * k == n:
        return (-im, re) if sign > 0 else (im, -re)
    wr = math.cos(2.0 * math.pi * k / n)
    wi = sign * math.sin(2.0 * math.pi * k / n)
    if 8 * k == n:
        c = wr
        if sign > 0:
            return (re - im) * c, (re + im) * c
        return (re + im) * c, (im - re) * c
    if 8 * k == 3 * n:
        c = -wr
        if sign > 0:
            return (-re - im) * c, (re - im) * c
        return (im - re) * c, (-re - im) * c
    return re * wr - im * wi, re * wi + im * wr


def _fft_list(xs, sign):
    n = len(xs)
    if n == 1:
        return xs
    ev = _fft_list(xs[0::2], sign)
    od = _fft_list(xs[1::2], sign)
    out = [None] * n
    for k in range(n // 2):
        tr, ti = _cmul_const(od[k], k, n, sign)
        er, ei = ev[k]
        out[k] = (er + tr, ei + ti)
        out[k + n // 2] = (er - tr, ei - ti)
    return out


def _dot(a, b):
    return jnp.dot(a, b, preferred_element_type=f32)


def _dot_nt(a, b):
    return lax.dot_general(a, b, (((1,), (1,)), ((), ())), preferred_element_type=f32)


def _ln_stats(x):
    m = jnp.mean(x, axis=0, keepdims=True)
    xc = x - m
    v = jnp.mean(xc * xc, axis=0, keepdims=True)
    return xc, lax.rsqrt(v + EPS)


def _ln_bwd(dn, n, r):
    m1 = jnp.mean(dn, axis=0, keepdims=True)
    m2 = jnp.mean(dn * n, axis=0, keepdims=True)
    return r * (dn - m1 - n * m2)


def _dft_d_fwd(v, cse_ref, cso_ref, flat_s, c0):
    top, bot = v[:DH], v[DH:]
    ze = _dot(cse_ref[...], (top + bot).astype(bf16))
    zo = _dot(cso_ref[...], (top - bot).astype(bf16))
    cols = pl.ds(c0, CC)
    flat_s[pl.ds(0, KE), cols] = ze[:KE]
    flat_s[pl.ds(KE, KO), cols] = zo[:KO]
    flat_s[pl.ds(KP, KE), cols] = ze[KE:]
    flat_s[pl.ds(KP + KE, KO), cols] = zo[KO:]


def _dft_d_inv(cset_ref, csot_ref, flat_s, c0):
    cols = pl.ds(c0, CC)
    ve = jnp.concatenate([flat_s[pl.ds(0, KE), cols], flat_s[pl.ds(KP, KE), cols]], axis=0)
    vo = jnp.concatenate([flat_s[pl.ds(KE, KO), cols], flat_s[pl.ds(KP + KE, KO), cols]], axis=0)
    ev = _dot(cset_ref[...], ve.astype(bf16))
    od = _dot(csot_ref[...], vo.astype(bf16))
    return jnp.concatenate([ev + od, ev - od], axis=0)


def _radix16(src_ref, dst_ref, sign, src_blocked, dst_blocked, extra=None):
    def body(j, carry):
        if extra is not None:
            idx = jnp.minimum(j, 2 * NB - 1)
            extra(idx // NB, pl.multiple_of((idx % NB) * BL, BL))
        r0 = pl.multiple_of(j * 8, 8)
        xs = []
        for a in range(NB):
            if src_blocked:
                re = src_ref[a, pl.ds(r0, 8), pl.ds(0, BL)]
                im = src_ref[a, pl.ds(r0, 8), pl.ds(BL, BL)]
            else:
                re = src_ref[pl.ds(r0, 8), pl.ds(a * BL, BL)]
                im = src_ref[pl.ds(KP + r0, 8), pl.ds(a * BL, BL)]
            xs.append((re, im))
        ys = _fft_list(xs, sign)
        for c in range(NB):
            re, im = ys[c]
            if dst_blocked:
                dst_ref[c, pl.ds(r0, 8), pl.ds(0, BL)] = re
                dst_ref[c, pl.ds(r0, 8), pl.ds(BL, BL)] = im
            else:
                dst_ref[pl.ds(r0, 8), pl.ds(c * BL, BL)] = re
                dst_ref[pl.ds(KP + r0, 8), pl.ds(c * BL, BL)] = im
        return carry
    lax.fori_loop(0, KP // 8, body, 0)


def _bins(ref, p, c):
    return jnp.concatenate([ref[p, c, pl.ds(0, KE, stride=2), :],
                            ref[p, c, pl.ds(1, KO, stride=2), :]], axis=0)


def _kernel(x_hbm, wr_hbm, wi_hbm, wg_hbm, wu_hbm, wdt_hbm, go_hbm,
            cse_ref, cso_ref, cset_hbm, csot_hbm, g_hbm, ck_ref,
            h2_hbm, dx_hbm, dwr_hbm, dwi_hbm, dwg_hbm, dwu_hbm, dwdt_hbm,
            flat_s, blk_s, xsp_s, wp_s, tmp_s, pad_s, h_s, n2_s, n2t_s, gon_s,
            ft_s, dn2t_s, dwg_s, dwu_s, dwdt_s,
            w_ref, go_ref, cset_ref, csot_ref, g_ref,
            h2_ref, dx_ref, dw_ref, x_ref, wbuf, dwbuf,
            in_sems, out_sems, x_sems, w_sems, dw_sems):
    step = pl.program_id(0)
    slot = step % 2

    def cp_x(j):
        return pltpu.make_async_copy(
            x_hbm.at[:, :, pl.ds(j * CC, CC)], x_ref.at[:, :, pl.ds(j * CC, CC)],
            x_sems.at[j])

    def cp_w(i, s):
        return [pltpu.make_async_copy(
            w.at[:, pl.ds(pl.multiple_of(i * FT, FT), FT)], wbuf.at[s, k], w_sems.at[s, k])
            for k, w in enumerate((wg_hbm, wu_hbm, wdt_hbm))]

    def cp_dw(i, s):
        return [pltpu.make_async_copy(
            dwbuf.at[s, k], w.at[:, pl.ds(pl.multiple_of(i * FT, FT), FT)], dw_sems.at[s, k])
            for k, w in enumerate((dwg_hbm, dwu_hbm, dwdt_hbm))]

    in_copies = [
        pltpu.make_async_copy(src, dst, in_sems.at[i])
        for i, (src, dst) in enumerate((
            (wr_hbm, w_ref.at[0]), (wi_hbm, w_ref.at[1]), (g_hbm, g_ref),
            (cset_hbm, cset_ref), (csot_hbm, csot_ref), (go_hbm, go_ref)))
    ]
    cp_wr, cp_wi, cp_g, cp_cset, cp_csot, cp_go = in_copies
    cp_h2 = pltpu.make_async_copy(h2_ref, h2_hbm, out_sems.at[0])
    cp_dwr = pltpu.make_async_copy(dw_ref.at[0], dwr_hbm, out_sems.at[1])
    cp_dwi = pltpu.make_async_copy(dw_ref.at[1], dwi_hbm, out_sems.at[2])

    def cp_dx(j):
        return pltpu.make_async_copy(
            dx_ref.at[:, :, pl.ds(j * CC, CC)], dx_hbm.at[:, :, pl.ds(j * CC, CC)],
            out_sems.at[3 + j])

    @pl.when(step == 0)
    def _phase_a():
        for j in range(NCC):
            cp_x(j).start()

        def ln1(j, carry):
            c0 = pl.multiple_of(j * CC, CC)
            cp_x(j).wait()

            @pl.when(j == NCC - 1)
            def _():
                for cp in in_copies + cp_w(0, 0):
                    cp.start()

            x = x_ref[0, :, pl.ds(c0, CC)].astype(f32)
            xc, r = _ln_stats(x)
            n1 = (xc * r).astype(bf16).astype(f32)
            _dft_d_fwd(n1, cse_ref, cso_ref, flat_s, c0)
            return carry
        lax.fori_loop(0, NCC, ln1, 0)

        _radix16(flat_s, blk_s, -1, False, True)

        cp_wr.wait()
        cp_wi.wait()
        pad_s[...] = jnp.zeros(pad_s.shape, f32)
        pad_s[:, pl.ds(0, DF - 256), :] = w_ref[:, pl.ds(256, DF - 256), :].astype(f32)
        for p in range(2):
            for l in range(NL):
                if l < NL - 1:
                    tmp_s[p, l] = w_ref[p, pl.ds(l * 128, 128), :].astype(f32).T
                else:
                    tmp_s[p, l] = pad_s[p].T
        cp_g.wait()

        def spec(c, carry):
            for p in range(2):
                for l in range(NL):
                    wp_s[p, c, pl.ds(l * 128, 128), :] = (
                        tmp_s[p, l, pl.ds(c, BL, stride=NB), :].T)
            ck = ck_ref[...]
            xx = _dot(blk_s[c].astype(bf16), g_ref[c])
            xsp_s[c] = xx
            xr, xi = xx[:, :BL], xx[:, BL:]
            wr = _bins(wp_s, 0, c) * ck
            wi = _bins(wp_s, 1, c) * ck
            yr = xr * wr - xi * wi
            yi = xr * wi + xi * wr
            y = jnp.concatenate([yr, yi], axis=1).astype(bf16)
            blk_s[c] = _dot_nt(y, g_ref[c])
            return carry
        lax.fori_loop(0, NB, spec, 0, unroll=2)

        _radix16(blk_s, flat_s, 1, True, False)
        cp_cset.wait()
        cp_csot.wait()
        cp_go.wait()

        def ln2(j, carry):
            c0 = pl.multiple_of(j * CC, CC)
            y = _dft_d_inv(cset_ref, csot_ref, flat_s, c0)
            h = x_ref[0, :, pl.ds(c0, CC)].astype(f32) + y
            h_s[:, pl.ds(c0, CC)] = h
            hc, r = _ln_stats(h)
            n2 = hc * r
            n2t_s[:, pl.ds(c0, CC)] = n2.astype(bf16)
            n2_s[pl.ds(c0, CC), :] = n2.T.astype(bf16)
            gon_s[pl.ds(c0, CC), :] = go_ref[0, :, pl.ds(c0, CC)].astype(f32).T.astype(bf16)
            return carry
        lax.fori_loop(0, NCC, ln2, 0)

    for cp in cp_w(step, slot):
        cp.wait()

    @pl.when(step + 1 < NF)
    def _():
        for cp in cp_w(step + 1, 1 - slot):
            cp.start()

    @pl.when(step >= 2)
    def _():
        for cp in cp_dw(step - 2, slot):
            cp.wait()

    wg_ref, wu_ref, wdt_ref = (wbuf.at[slot, k] for k in range(3))
    dwg_ref, dwu_ref, dwdt_ref = (dwbuf.at[slot, k] for k in range(3))

    def chunk(j, carry):
        r0 = pl.multiple_of(j * TM, TM)
        n2c = n2_s[pl.ds(r0, TM), :]
        goc = gon_s[pl.ds(r0, TM), :]
        wg = wg_ref[...]
        wu = wu_ref[...]
        wdt = wdt_ref[...]
        a = _dot(n2c, wg)
        u = _dot(n2c, wu)
        dgu = _dot(goc, wdt)
        sig = jax.nn.sigmoid(a)
        g = a * sig
        gu = (g * u).astype(bf16)
        du = (dgu * g).astype(bf16)
        da = (dgu * u * (sig * (1.0 + a * (1.0 - sig)))).astype(bf16)
        ft_s[:, pl.ds(r0, TM)] = (
            jnp.where(step > 0, ft_s[:, pl.ds(r0, TM)], 0.0) + _dot_nt(wdt, gu))
        dn2t_s[:, pl.ds(r0, TM)] = (
            jnp.where(step > 0, dn2t_s[:, pl.ds(r0, TM)], 0.0)
            + _dot_nt(wg, da) + _dot_nt(wu, du))
        n2tc = n2t_s[:, pl.ds(r0, TM)]
        for acc_s, o_ref, lhs, rhs in (
                (dwg_s, dwg_ref, n2tc, da), (dwu_s, dwu_ref, n2tc, du),
                (dwdt_s, dwdt_ref, go_ref[0, :, pl.ds(r0, TM)], gu)):
            acc = jnp.where(j > 0, acc_s[...], 0.0) + _dot(lhs, rhs)
            acc_s[...] = acc
            o_ref[...] = acc.astype(bf16)
        return carry
    lax.fori_loop(0, S // TM, chunk, 0)
    for cp in cp_dw(step, slot):
        cp.start()

    @pl.when(step == NF - 1)
    def _phase_c():
        def ln2b(j, carry):
            c0 = pl.multiple_of(j * CC, CC)
            h = h_s[:, pl.ds(c0, CC)]
            h2_ref[0, :, pl.ds(c0, CC)] = (h + ft_s[:, pl.ds(c0, CC)]).astype(bf16)
            hc, r = _ln_stats(h)
            dn2 = dn2t_s[:, pl.ds(c0, CC)]
            dh = go_ref[0, :, pl.ds(c0, CC)].astype(f32) + _ln_bwd(dn2, hc * r, r)
            h_s[:, pl.ds(c0, CC)] = dh
            _dft_d_fwd(dh, cse_ref, cso_ref, flat_s, c0)
            return carry
        lax.fori_loop(0, NCC, ln2b, 0)
        cp_h2.start()

        _radix16(flat_s, blk_s, -1, False, True)

        def specb(c, carry):
            ck = ck_ref[...]
            gy = _dot(blk_s[c].astype(bf16), g_ref[c])
            gyr = gy[:, :BL] * ck
            gyi = gy[:, BL:] * ck
            xx = xsp_s[c]
            xr, xi = xx[:, :BL], xx[:, BL:]
            wr = _bins(wp_s, 0, c)
            wi = _bins(wp_s, 1, c)
            gxr = gyr * wr + gyi * wi
            gxi = gyi * wr - gyr * wi
            gx = jnp.concatenate([gxr, gxi], axis=1).astype(bf16)
            blk_s[c] = _dot_nt(gx, g_ref[c])
            dws = (gyr * xr + gyi * xi, gyi * xr - gyr * xi)
            for p in range(2):
                wp_s[p, c, pl.ds(0, KE, stride=2), :] = dws[p][:KE]
                wp_s[p, c, pl.ds(1, KO, stride=2), :] = dws[p][KE:]
                for l in range(NL):
                    tmp_s[p, l, pl.ds(c, BL, stride=NB), :] = (
                        wp_s[p, c, pl.ds(l * 128, 128), :].T)
            return carry
        lax.fori_loop(0, NB, specb, 0, unroll=2)

        for p in range(2):
            for l in range(NL):
                n = min(128, DF - l * 128)
                dw_ref[p, pl.ds(l * 128, n), :] = tmp_s[p, l].T[:n].astype(bf16)
            (cp_dwr, cp_dwi)[p].start()

        _radix16(blk_s, flat_s, 1, True, False)

        def ln1b(j, carry):
            c0 = pl.multiple_of(j * CC, CC)
            dn1 = _dft_d_inv(cset_ref, csot_ref, flat_s, c0)
            x = x_ref[0, :, pl.ds(c0, CC)].astype(f32)
            xc, r = _ln_stats(x)
            dx = h_s[:, pl.ds(c0, CC)] + _ln_bwd(dn1, xc * r, r)
            dx_ref[0, :, pl.ds(c0, CC)] = dx.astype(bf16)
            cp_dx(j).start()
            return carry
        lax.fori_loop(0, NCC, ln1b, 0)
        cp_h2.wait()
        cp_dwr.wait()
        cp_dwi.wait()
        for j in range(NCC):
            cp_dx(j).wait()
        for cp in cp_dw(NF - 2, (NF - 2) % 2) + cp_dw(NF - 1, (NF - 1) % 2):
            cp.wait()


@jax.jit
def pallas_sequential_preLN__spectral_gfnet__swiglu_ffn__prompt_kernel(
    A_x: jax.Array,
    A_w_r: jax.Array,
    A_w_i: jax.Array,
    B_x: jax.Array,
    B_w_gate: jax.Array,
    B_w_up: jax.Array,
    B_w_down: jax.Array,
    grad_out: jax.Array,
):
    del B_x
    cse = jnp.asarray(_CSE, dtype=bf16)
    cso = jnp.asarray(_CSO, dtype=bf16)
    cset = jnp.asarray(_CSET, dtype=bf16)
    csot = jnp.asarray(_CSOT, dtype=bf16)
    g = jnp.asarray(_G, dtype=bf16)
    ck = jnp.asarray(_CK, dtype=f32)

    xt = jnp.swapaxes(A_x, 1, 2)
    got = jnp.swapaxes(grad_out, 1, 2)
    wrt = A_w_r.T
    wit = A_w_i.T
    wdt = B_w_down.T

    def whole(shape):
        nd = len(shape)
        return pl.BlockSpec(shape, lambda i: (0,) * nd, pipeline_mode=pl.Buffered(1))

    hbm = pl.BlockSpec(memory_space=pl.ANY)
    in_specs = [
        hbm,
        hbm,
        hbm,
        hbm,
        hbm,
        hbm,
        hbm,
        whole((2 * KE, DH)),
        whole((2 * KO, DH)),
        hbm,
        hbm,
        hbm,
        whole((KP, BL)),
    ]
    out_specs = [
        hbm, hbm, hbm, hbm, hbm, hbm, hbm,
    ]
    out_shape = [
        jax.ShapeDtypeStruct((1, D, S), bf16),
        jax.ShapeDtypeStruct((1, D, S), bf16),
        jax.ShapeDtypeStruct((DF, S), bf16),
        jax.ShapeDtypeStruct((DF, S), bf16),
        jax.ShapeDtypeStruct((D, F), bf16),
        jax.ShapeDtypeStruct((D, F), bf16),
        jax.ShapeDtypeStruct((D, F), bf16),
    ]
    scratch = [
        pltpu.VMEM((2 * KP, S), f32),
        pltpu.VMEM((NB, KP, 2 * BL), f32),
        pltpu.VMEM((NB, KP, 2 * BL), f32),
        pltpu.VMEM((2, NB, KL, BL), f32),
        pltpu.VMEM((2, NL, S, 128), f32),
        pltpu.VMEM((2, 128, S), f32),
        pltpu.VMEM((D, S), f32),
        pltpu.VMEM((S, D), bf16),
        pltpu.VMEM((D, S), bf16),
        pltpu.VMEM((S, D), bf16),
        pltpu.VMEM((D, S), f32),
        pltpu.VMEM((D, S), f32),
        pltpu.VMEM((D, FT), f32),
        pltpu.VMEM((D, FT), f32),
        pltpu.VMEM((D, FT), f32),
        pltpu.VMEM((2, DF, S), bf16),
        pltpu.VMEM((1, D, S), bf16),
        pltpu.VMEM((DH, 2 * KE), bf16),
        pltpu.VMEM((DH, 2 * KO), bf16),
        pltpu.VMEM((NB, 2 * BL, 2 * BL), bf16),
        pltpu.VMEM((1, D, S), bf16),
        pltpu.VMEM((1, D, S), bf16),
        pltpu.VMEM((2, DF, S), bf16),
        pltpu.VMEM((1, D, S), bf16),
        pltpu.VMEM((2, 3, D, FT), bf16),
        pltpu.VMEM((2, 3, D, FT), bf16),
        pltpu.SemaphoreType.DMA((6,)),
        pltpu.SemaphoreType.DMA((3 + NCC,)),
        pltpu.SemaphoreType.DMA((NCC,)),
        pltpu.SemaphoreType.DMA((2, 3)),
        pltpu.SemaphoreType.DMA((2, 3)),
    ]
    h2t, dxt, dwrt, dwit, dwg, dwu, dwdt = pl.pallas_call(
        _kernel,
        grid=(NF,),
        in_specs=in_specs,
        out_specs=out_specs,
        out_shape=out_shape,
        scratch_shapes=scratch,
        compiler_params=pltpu.CompilerParams(
            dimension_semantics=("arbitrary",),
            vmem_limit_bytes=110 * 1024 * 1024,
        ),
    )(xt, wrt, wit, B_w_gate, B_w_up, wdt, got, cse, cso, cset, csot, g, ck)
    return (jnp.swapaxes(h2t, 1, 2), jnp.swapaxes(dxt, 1, 2), dwrt.T, dwit.T,
            dwg, dwu, dwdt.T)
```

```python
import math

import numpy as np
import jax
import jax.numpy as jnp
from jax import lax
import jax.experimental.pallas as pl
import jax.experimental.pallas.tpu as pltpu

S = 2048
D = 576
F = 4608
DH = D // 2
DF = D // 2 + 1
KE = 160
KO = 144
KP = KE + KO
KL = 384
NB = 16
BL = 128
NL = KL // 128
EPS = 1e-5

FT = 512
TM = 512
NF = F // FT
CC = 1024
NCC = S // CC

f32 = jnp.float32
bf16 = jnp.bfloat16


def _make_consts():
    d = np.arange(DH)[None, :]
    ke = np.arange(0, DF, 2)[:, None]
    ko = np.arange(1, DF, 2)[:, None]
    ae = 2.0 * np.pi * ((d * ke) % D) / D
    ao = 2.0 * np.pi * ((d * ko) % D) / D
    cse = np.zeros((2 * KE, DH), np.float64)
    cse[:ke.shape[0]] = np.cos(ae)
    cse[KE:KE + ke.shape[0]] = -np.sin(ae)
    cso = np.concatenate([np.cos(ao), -np.sin(ao)], axis=0)
    g = np.zeros((NB, 2 * BL, 2 * BL), np.float64)
    b = np.arange(BL)[:, None]
    e = np.arange(BL)[None, :]
    for c in range(NB):
        th = 2.0 * np.pi * ((b * (c + NB * e)) % S) / S
        cm, sm = np.cos(th), np.sin(th)
        g[c, :BL, :BL] = cm
        g[c, :BL, BL:] = -sm
        g[c, BL:, :BL] = sm
        g[c, BL:, BL:] = cm
    ck = np.zeros((KP, BL), np.float64)
    ck[:ke.shape[0]] = 2.0
    ck[KE:] = 2.0
    ck[0] = 1.0
    ck[ke.shape[0] - 1] = 1.0
    ck = ck / (S * D)
    c32 = lambda a: np.ascontiguousarray(a).astype(np.float32)
    return c32(cse), c32(cso), c32(cse.T), c32(cso.T), c32(g), c32(ck)


_CSE, _CSO, _CSET, _CSOT, _G, _CK = _make_consts()


def _cmul_const(z, k, n, sign):
    re, im = z
    k = k % n
    if k == 0:
        return re, im
    if 4 * k == n:
        return (-im, re) if sign > 0 else (im, -re)
    wr = math.cos(2.0 * math.pi * k / n)
    wi = sign * math.sin(2.0 * math.pi * k / n)
    if 8 * k == n:
        c = wr
        if sign > 0:
            return (re - im) * c, (re + im) * c
        return (re + im) * c, (im - re) * c
    if 8 * k == 3 * n:
        c = -wr
        if sign > 0:
            return (-re - im) * c, (re - im) * c
        return (im - re) * c, (-re - im) * c
    return re * wr - im * wi, re * wi + im * wr


def _fft_list(xs, sign):
    n = len(xs)
    if n == 1:
        return xs
    ev = _fft_list(xs[0::2], sign)
    od = _fft_list(xs[1::2], sign)
    out = [None] * n
    for k in range(n // 2):
        tr, ti = _cmul_const(od[k], k, n, sign)
        er, ei = ev[k]
        out[k] = (er + tr, ei + ti)
        out[k + n // 2] = (er - tr, ei - ti)
    return out


def _dot(a, b):
    return jnp.dot(a, b, preferred_element_type=f32)


def _dot_nt(a, b):
    return lax.dot_general(a, b, (((1,), (1,)), ((), ())), preferred_element_type=f32)


def _ln_stats(x):
    m = jnp.mean(x, axis=0, keepdims=True)
    xc = x - m
    v = jnp.mean(xc * xc, axis=0, keepdims=True)
    return m, xc, lax.rsqrt(v + EPS)


def _ln_bwd(dn, n, r):
    m1 = jnp.mean(dn, axis=0, keepdims=True)
    m2 = jnp.mean(dn * n, axis=0, keepdims=True)
    return r * (dn - m1 - n * m2)


def _dft_d_fwd(v, cse_ref, cso_ref, flat_s, c0):
    top, bot = v[:DH], v[DH:]
    ze = _dot(cse_ref[...], (top + bot).astype(bf16))
    zo = _dot(cso_ref[...], (top - bot).astype(bf16))
    cols = pl.ds(c0, CC)
    flat_s[pl.ds(0, KE), cols] = ze[:KE]
    flat_s[pl.ds(KE, KO), cols] = zo[:KO]
    flat_s[pl.ds(KP, KE), cols] = ze[KE:]
    flat_s[pl.ds(KP + KE, KO), cols] = zo[KO:]


def _dft_d_inv(cset_ref, csot_ref, flat_s, c0):
    cols = pl.ds(c0, CC)
    ve = jnp.concatenate([flat_s[pl.ds(0, KE), cols], flat_s[pl.ds(KP, KE), cols]], axis=0)
    vo = jnp.concatenate([flat_s[pl.ds(KE, KO), cols], flat_s[pl.ds(KP + KE, KO), cols]], axis=0)
    ev = _dot(cset_ref[...], ve.astype(bf16))
    od = _dot(csot_ref[...], vo.astype(bf16))
    return jnp.concatenate([ev + od, ev - od], axis=0)


def _radix16(src_ref, dst_ref, sign, src_blocked, dst_blocked):
    def body(j, carry):
        r0 = pl.multiple_of(j * 8, 8)
        xs = []
        for a in range(NB):
            if src_blocked:
                re = src_ref[a, pl.ds(r0, 8), pl.ds(0, BL)]
                im = src_ref[a, pl.ds(r0, 8), pl.ds(BL, BL)]
            else:
                re = src_ref[pl.ds(r0, 8), pl.ds(a * BL, BL)]
                im = src_ref[pl.ds(KP + r0, 8), pl.ds(a * BL, BL)]
            xs.append((re, im))
        ys = _fft_list(xs, sign)
        for c in range(NB):
            re, im = ys[c]
            if dst_blocked:
                dst_ref[c, pl.ds(r0, 8), pl.ds(0, BL)] = re
                dst_ref[c, pl.ds(r0, 8), pl.ds(BL, BL)] = im
            else:
                dst_ref[pl.ds(r0, 8), pl.ds(c * BL, BL)] = re
                dst_ref[pl.ds(KP + r0, 8), pl.ds(c * BL, BL)] = im
        return carry
    lax.fori_loop(0, KP // 8, body, 0, unroll=2)


def _bins(ref, p, c):
    return jnp.concatenate([ref[p, c, pl.ds(0, KE, stride=2), :],
                            ref[p, c, pl.ds(1, KO, stride=2), :]], axis=0)


def _kernel(x_hbm, wr_hbm, wi_hbm, wg_hbm, wu_hbm, wdt_hbm, go_hbm,
            cse_ref, cso_ref, cset_hbm, csot_hbm, g_hbm, ck_ref,
            h2_hbm, dx_hbm, dwr_hbm, dwi_hbm, dwg_hbm, dwu_hbm, dwdt_hbm,
            flat_s, blk_s, xsp_s, wp_s, tmp_s, pad_s, h_s, n2_s, n2t_s, gon_s,
            ft_s, dn2t_s, dwg_s, dwu_s, dwdt_s, st_s,
            w_ref, go_ref, cset_ref, csot_ref, g_ref,
            h2_ref, dx_ref, dw_ref, x_ref, wbuf, dwbuf,
            in_sems, out_sems, x_sems, w_sems, dw_sems):
    step = pl.program_id(0)
    slot = step % 2

    def cp_x(j):
        return pltpu.make_async_copy(
            x_hbm.at[:, :, pl.ds(j * CC, CC)], x_ref.at[:, :, pl.ds(j * CC, CC)],
            x_sems.at[j])

    def cp_w(i, s):
        return [pltpu.make_async_copy(
            w.at[:, pl.ds(pl.multiple_of(i * FT, FT), FT)], wbuf.at[s, k], w_sems.at[s, k])
            for k, w in enumerate((wg_hbm, wu_hbm, wdt_hbm))]

    def cp_dw(i, s):
        return [pltpu.make_async_copy(
            dwbuf.at[s, k], w.at[:, pl.ds(pl.multiple_of(i * FT, FT), FT)], dw_sems.at[s, k])
            for k, w in enumerate((dwg_hbm, dwu_hbm, dwdt_hbm))]

    in_copies = [
        pltpu.make_async_copy(src, dst, in_sems.at[i])
        for i, (src, dst) in enumerate((
            (wr_hbm, w_ref.at[0]), (wi_hbm, w_ref.at[1]), (g_hbm, g_ref),
            (cset_hbm, cset_ref), (csot_hbm, csot_ref), (go_hbm, go_ref)))
    ]
    cp_wr, cp_wi, cp_g, cp_cset, cp_csot, cp_go = in_copies
    cp_h2 = pltpu.make_async_copy(h2_ref, h2_hbm, out_sems.at[0])
    cp_dwr = pltpu.make_async_copy(dw_ref.at[0], dwr_hbm, out_sems.at[1])
    cp_dwi = pltpu.make_async_copy(dw_ref.at[1], dwi_hbm, out_sems.at[2])

    def cp_dx(j):
        return pltpu.make_async_copy(
            dx_ref.at[:, :, pl.ds(j * CC, CC)], dx_hbm.at[:, :, pl.ds(j * CC, CC)],
            out_sems.at[3 + j])

    @pl.when(step == 0)
    def _phase_a():
        for j in range(NCC):
            cp_x(j).start()

        def ln1(j, carry):
            c0 = pl.multiple_of(j * CC, CC)
            cp_x(j).wait()

            @pl.when(j == NCC - 1)
            def _():
                for cp in in_copies + cp_w(0, 0):
                    cp.start()

            x = x_ref[0, :, pl.ds(c0, CC)].astype(f32)
            m, xc, r = _ln_stats(x)
            st_s[pl.ds(0, 1), pl.ds(c0, CC)] = m
            st_s[pl.ds(1, 1), pl.ds(c0, CC)] = r
            n1 = (xc * r).astype(bf16).astype(f32)
            _dft_d_fwd(n1, cse_ref, cso_ref, flat_s, c0)
            return carry
        lax.fori_loop(0, NCC, ln1, 0)

        _radix16(flat_s, blk_s, -1, False, True)

        cp_wr.wait()
        cp_wi.wait()
        pad_s[...] = jnp.zeros(pad_s.shape, f32)
        pad_s[:, pl.ds(0, DF - 256), :] = w_ref[:, pl.ds(256, DF - 256), :].astype(f32)
        for p in range(2):
            for l in range(NL):
                if l < NL - 1:
                    tmp_s[p, l] = w_ref[p, pl.ds(l * 128, 128), :].astype(f32).T
                else:
                    tmp_s[p, l] = pad_s[p].T
        cp_g.wait()

        def spec(c, carry):
            for p in range(2):
                for l in range(NL):
                    wp_s[p, c, pl.ds(l * 128, 128), :] = (
                        tmp_s[p, l, pl.ds(c, BL, stride=NB), :].T)
            ck = ck_ref[...]
            xx = _dot(blk_s[c].astype(bf16), g_ref[c])
            xsp_s[c] = xx
            xr, xi = xx[:, :BL], xx[:, BL:]
            wr = _bins(wp_s, 0, c) * ck
            wi = _bins(wp_s, 1, c) * ck
            yr = xr * wr - xi * wi
            yi = xr * wi + xi * wr
            y = jnp.concatenate([yr, yi], axis=1).astype(bf16)
            blk_s[c] = _dot_nt(y, g_ref[c])
            return carry
        lax.fori_loop(0, NB, spec, 0, unroll=2)

        _radix16(blk_s, flat_s, 1, True, False)
        cp_cset.wait()
        cp_csot.wait()
        cp_go.wait()

        def ln2(j, carry):
            c0 = pl.multiple_of(j * CC, CC)
            y = _dft_d_inv(cset_ref, csot_ref, flat_s, c0)
            h = x_ref[0, :, pl.ds(c0, CC)].astype(f32) + y
            h_s[:, pl.ds(c0, CC)] = h
            m, hc, r = _ln_stats(h)
            st_s[pl.ds(2, 1), pl.ds(c0, CC)] = m
            st_s[pl.ds(3, 1), pl.ds(c0, CC)] = r
            n2 = hc * r
            n2t_s[:, pl.ds(c0, CC)] = n2.astype(bf16)
            n2_s[pl.ds(c0, CC), :] = n2.T.astype(bf16)
            gon_s[pl.ds(c0, CC), :] = go_ref[0, :, pl.ds(c0, CC)].astype(f32).T.astype(bf16)
            return carry
        lax.fori_loop(0, NCC, ln2, 0)

    for cp in cp_w(step, slot):
        cp.wait()

    @pl.when(step + 1 < NF)
    def _():
        for cp in cp_w(step + 1, 1 - slot):
            cp.start()

    @pl.when(step >= 2)
    def _():
        for cp in cp_dw(step - 2, slot):
            cp.wait()

    wg_ref, wu_ref, wdt_ref = (wbuf.at[slot, k] for k in range(3))
    dwg_ref, dwu_ref, dwdt_ref = (dwbuf.at[slot, k] for k in range(3))

    def chunk(j, carry):
        r0 = pl.multiple_of(j * TM, TM)
        n2c = n2_s[pl.ds(r0, TM), :]
        goc = gon_s[pl.ds(r0, TM), :]
        wg = wg_ref[...]
        wu = wu_ref[...]
        wdt = wdt_ref[...]
        a = _dot(n2c, wg)
        u = _dot(n2c, wu)
        dgu = _dot(goc, wdt)
        sig = jax.nn.sigmoid(a)
        g = a * sig
        gu = (g * u).astype(bf16)
        du = (dgu * g).astype(bf16)
        da = (dgu * u * (sig * (1.0 + a * (1.0 - sig)))).astype(bf16)
        ft_s[:, pl.ds(r0, TM)] = (
            jnp.where(step > 0, ft_s[:, pl.ds(r0, TM)], 0.0) + _dot_nt(wdt, gu))
        dn2t_s[:, pl.ds(r0, TM)] = (
            jnp.where(step > 0, dn2t_s[:, pl.ds(r0, TM)], 0.0)
            + _dot_nt(wg, da) + _dot_nt(wu, du))
        n2tc = n2t_s[:, pl.ds(r0, TM)]
        for acc_s, o_ref, lhs, rhs in (
                (dwg_s, dwg_ref, n2tc, da), (dwu_s, dwu_ref, n2tc, du),
                (dwdt_s, dwdt_ref, go_ref[0, :, pl.ds(r0, TM)], gu)):
            acc = jnp.where(j > 0, acc_s[...], 0.0) + _dot(lhs, rhs)
            acc_s[...] = acc
            o_ref[...] = acc.astype(bf16)
        return carry
    lax.fori_loop(0, S // TM, chunk, 0)
    for cp in cp_dw(step, slot):
        cp.start()

    @pl.when(step == NF - 1)
    def _phase_c():
        def ln2b(j, carry):
            c0 = pl.multiple_of(j * CC, CC)
            h = h_s[:, pl.ds(c0, CC)]
            h2_ref[0, :, pl.ds(c0, CC)] = (h + ft_s[:, pl.ds(c0, CC)]).astype(bf16)
            m = st_s[pl.ds(2, 1), pl.ds(c0, CC)]
            r = st_s[pl.ds(3, 1), pl.ds(c0, CC)]
            dn2 = dn2t_s[:, pl.ds(c0, CC)]
            dh = go_ref[0, :, pl.ds(c0, CC)].astype(f32) + _ln_bwd(dn2, (h - m) * r, r)
            h_s[:, pl.ds(c0, CC)] = dh
            _dft_d_fwd(dh, cse_ref, cso_ref, flat_s, c0)
            return carry
        lax.fori_loop(0, NCC, ln2b, 0)
        cp_h2.start()

        _radix16(flat_s, blk_s, -1, False, True)

        def specb(c, carry):
            ck = ck_ref[...]
            gy = _dot(blk_s[c].astype(bf16), g_ref[c])
            gyr = gy[:, :BL] * ck
            gyi = gy[:, BL:] * ck
            xx = xsp_s[c]
            xr, xi = xx[:, :BL], xx[:, BL:]
            wr = _bins(wp_s, 0, c)
            wi = _bins(wp_s, 1, c)
            gxr = gyr * wr + gyi * wi
            gxi = gyi * wr - gyr * wi
            gx = jnp.concatenate([gxr, gxi], axis=1).astype(bf16)
            blk_s[c] = _dot_nt(gx, g_ref[c])
            dws = (gyr * xr + gyi * xi, gyi * xr - gyr * xi)
            for p in range(2):
                wp_s[p, c, pl.ds(0, KE, stride=2), :] = dws[p][:KE]
                wp_s[p, c, pl.ds(1, KO, stride=2), :] = dws[p][KE:]
                for l in range(NL):
                    tmp_s[p, l, pl.ds(c, BL, stride=NB), :] = (
                        wp_s[p, c, pl.ds(l * 128, 128), :].T)
            return carry
        lax.fori_loop(0, NB, specb, 0, unroll=2)

        for p in range(2):
            for l in range(NL):
                n = min(128, DF - l * 128)
                dw_ref[p, pl.ds(l * 128, n), :] = tmp_s[p, l].T[:n].astype(bf16)
            (cp_dwr, cp_dwi)[p].start()

        _radix16(blk_s, flat_s, 1, True, False)

        def ln1b(j, carry):
            c0 = pl.multiple_of(j * CC, CC)
            dn1 = _dft_d_inv(cset_ref, csot_ref, flat_s, c0)
            x = x_ref[0, :, pl.ds(c0, CC)].astype(f32)
            m = st_s[pl.ds(0, 1), pl.ds(c0, CC)]
            r = st_s[pl.ds(1, 1), pl.ds(c0, CC)]
            dx = h_s[:, pl.ds(c0, CC)] + _ln_bwd(dn1, (x - m) * r, r)
            dx_ref[0, :, pl.ds(c0, CC)] = dx.astype(bf16)
            cp_dx(j).start()
            return carry
        lax.fori_loop(0, NCC, ln1b, 0)
        cp_h2.wait()
        cp_dwr.wait()
        cp_dwi.wait()
        for j in range(NCC):
            cp_dx(j).wait()
        for cp in cp_dw(NF - 2, (NF - 2) % 2) + cp_dw(NF - 1, (NF - 1) % 2):
            cp.wait()


@jax.jit
def pallas_sequential_preLN__spectral_gfnet__swiglu_ffn__prompt_kernel(
    A_x: jax.Array,
    A_w_r: jax.Array,
    A_w_i: jax.Array,
    B_x: jax.Array,
    B_w_gate: jax.Array,
    B_w_up: jax.Array,
    B_w_down: jax.Array,
    grad_out: jax.Array,
):
    del B_x
    cse = jnp.asarray(_CSE, dtype=bf16)
    cso = jnp.asarray(_CSO, dtype=bf16)
    cset = jnp.asarray(_CSET, dtype=bf16)
    csot = jnp.asarray(_CSOT, dtype=bf16)
    g = jnp.asarray(_G, dtype=bf16)
    ck = jnp.asarray(_CK, dtype=f32)

    xt = jnp.swapaxes(A_x, 1, 2)
    got = jnp.swapaxes(grad_out, 1, 2)
    wrt = A_w_r.T
    wit = A_w_i.T
    wdt = B_w_down.T

    def whole(shape):
        nd = len(shape)
        return pl.BlockSpec(shape, lambda i: (0,) * nd, pipeline_mode=pl.Buffered(1))

    hbm = pl.BlockSpec(memory_space=pl.ANY)
    in_specs = [
        hbm,
        hbm,
        hbm,
        hbm,
        hbm,
        hbm,
        hbm,
        whole((2 * KE, DH)),
        whole((2 * KO, DH)),
        hbm,
        hbm,
        hbm,
        whole((KP, BL)),
    ]
    out_specs = [
        hbm, hbm, hbm, hbm, hbm, hbm, hbm,
    ]
    out_shape = [
        jax.ShapeDtypeStruct((1, D, S), bf16),
        jax.ShapeDtypeStruct((1, D, S), bf16),
        jax.ShapeDtypeStruct((DF, S), bf16),
        jax.ShapeDtypeStruct((DF, S), bf16),
        jax.ShapeDtypeStruct((D, F), bf16),
        jax.ShapeDtypeStruct((D, F), bf16),
        jax.ShapeDtypeStruct((D, F), bf16),
    ]
    scratch = [
        pltpu.VMEM((2 * KP, S), f32),
        pltpu.VMEM((NB, KP, 2 * BL), f32),
        pltpu.VMEM((NB, KP, 2 * BL), f32),
        pltpu.VMEM((2, NB, KL, BL), f32),
        pltpu.VMEM((2, NL, S, 128), f32),
        pltpu.VMEM((2, 128, S), f32),
        pltpu.VMEM((D, S), f32),
        pltpu.VMEM((S, D), bf16),
        pltpu.VMEM((D, S), bf16),
        pltpu.VMEM((S, D), bf16),
        pltpu.VMEM((D, S), f32),
        pltpu.VMEM((D, S), f32),
        pltpu.VMEM((D, FT), f32),
        pltpu.VMEM((D, FT), f32),
        pltpu.VMEM((D, FT), f32),
        pltpu.VMEM((8, S), f32),
        pltpu.VMEM((2, DF, S), bf16),
        pltpu.VMEM((1, D, S), bf16),
        pltpu.VMEM((DH, 2 * KE), bf16),
        pltpu.VMEM((DH, 2 * KO), bf16),
        pltpu.VMEM((NB, 2 * BL, 2 * BL), bf16),
        pltpu.VMEM((1, D, S), bf16),
        pltpu.VMEM((1, D, S), bf16),
        pltpu.VMEM((2, DF, S), bf16),
        pltpu.VMEM((1, D, S), bf16),
        pltpu.VMEM((2, 3, D, FT), bf16),
        pltpu.VMEM((2, 3, D, FT), bf16),
        pltpu.SemaphoreType.DMA((6,)),
        pltpu.SemaphoreType.DMA((3 + NCC,)),
        pltpu.SemaphoreType.DMA((NCC,)),
        pltpu.SemaphoreType.DMA((2, 3)),
        pltpu.SemaphoreType.DMA((2, 3)),
    ]
    h2t, dxt, dwrt, dwit, dwg, dwu, dwdt = pl.pallas_call(
        _kernel,
        grid=(NF,),
        in_specs=in_specs,
        out_specs=out_specs,
        out_shape=out_shape,
        scratch_shapes=scratch,
        compiler_params=pltpu.CompilerParams(
            dimension_semantics=("arbitrary",),
            vmem_limit_bytes=110 * 1024 * 1024,
        ),
    )(xt, wrt, wit, B_w_gate, B_w_up, wdt, got, cse, cso, cset, csot, g, ck)
    return (jnp.swapaxes(h2t, 1, 2), jnp.swapaxes(dxt, 1, 2), dwrt.T, dwit.T,
            dwg, dwu, dwdt.T)
```
